```python
import os as _os
_os.environ.setdefault("JAX_PLATFORMS", "cpu")
import jax
import jax.numpy as jnp

def _softmax(x, axis=-1):
    return jax.nn.softmax(x, axis=axis)
def _gelu(x):
    return jax.nn.gelu(x, approximate=True)
def _silu(x):
    return jax.nn.silu(x)
def _sigmoid(x):
    return jax.nn.sigmoid(x)
def _layernorm(x, axis=-1, eps=1e-5):
    m = jnp.mean(x, axis=axis, keepdims=True)
    v = jnp.var(x, axis=axis, keepdims=True)
    return (x - m) / jnp.sqrt(v + eps)
def _scatter_add(tgt, idx, src, axis=0):
    return tgt.at[idx].add(src)
def _segment_sum(src, seg, n):
    return jax.ops.segment_sum(src, seg, n)
class _Rng:
    def __init__(self, key):
        self._k = key
    def _next(self):
        self._k, sub = jax.random.split(self._k)
        return sub
    def normal(self, shape):
        return jax.random.normal(self._next(), shape, dtype=jnp.bfloat16)
    def randint(self, lo, hi, shape):
        return jax.random.randint(self._next(), shape, lo, hi, dtype=jnp.int32)
    def uniform(self, shape, lo=0.0, hi=1.0):
        return jax.random.uniform(self._next(), shape, jnp.bfloat16, lo, hi)
    def permutation(self, n):
        return jax.random.permutation(self._next(), n)


kernel_name = 'concat_heads__mha_block_cached__mha_block_cached__near_ridge'

def setup_inputs():
    _rng = _Rng(jax.random.key(int.from_bytes(__import__("os").urandom(4), "little")))
    _w = (lambda a: (lambda t: t.astype(jnp.bfloat16) if jnp.issubdtype(t.dtype, jnp.floating) else t)(jnp.asarray(a)))
    def _A_setup():
        B, Sq, D = 32, 32, 640
        H, Sk, Dh = 32, 32, 128
        return {
            "x": _w((lambda *s: _rng.normal(s) * 0.8)(B, Sq, D)),
            "k_cache": _w((lambda *s: _rng.normal(s) * 0.8)(B, H, Sk, Dh)),
            "v_cache": _w((lambda *s: _rng.normal(s) * 0.05)(B, H, Sk, Dh)),
            "wq": _w((lambda *s: _rng.normal(s) * 0.8)(D, H * Dh) * (D ** -0.5)),
            "wo": _w((lambda *s: _rng.normal(s) * 0.05)(H * Dh, D) * ((H * Dh) ** -0.5)),
        }
    _A_in = _A_setup()

    def _B_setup():
        B, Sq, D = 32, 32, 640
        H, Sk, Dh = 32, 32, 128
        return {
            "x": _w((lambda *s: _rng.normal(s) * 0.8)(B, Sq, D)),
            "k_cache": _w((lambda *s: _rng.normal(s) * 0.8)(B, H, Sk, Dh)),
            "v_cache": _w((lambda *s: _rng.normal(s) * 0.05)(B, H, Sk, Dh)),
            "wq": _w((lambda *s: _rng.normal(s) * 0.8)(D, H * Dh) * (D ** -0.5)),
            "wo": _w((lambda *s: _rng.normal(s) * 0.05)(H * Dh, D) * ((H * Dh) ** -0.5)),
        }
    _B_in = _B_setup()

    return {
        "A_x": _A_in["x"],
        "A_k_cache": _A_in["k_cache"],
        "A_v_cache": _A_in["v_cache"],
        "A_wq": _A_in["wq"],
        "A_wo": _A_in["wo"],
        "B_x": _B_in["x"],
        "B_k_cache": _B_in["k_cache"],
        "B_v_cache": _B_in["v_cache"],
        "B_wq": _B_in["wq"],
        "B_wo": _B_in["wo"],
    }

def reference(A_x, A_k_cache, A_v_cache, A_wq, A_wo, B_x, B_k_cache, B_v_cache, B_wq, B_wo):
    def _A_ref(x, k_cache, v_cache, wq, wo):
        B, Sq, D = x.shape
        H, Dh = 32, 128
        q = (lambda x, *d: x.transpose(*d))((x @ wq).reshape(B, Sq, H, Dh), 0, 2, 1, 3)
        scores = jnp.einsum("bhqd,bhkd->bhqk", q, k_cache) * (Dh ** -0.5)
        p = _softmax(scores, axis=-1)
        o = jnp.einsum("bhqk,bhkd->bhqd", p, v_cache)
        return (lambda x, *d: x.transpose(*d))(o, 0, 2, 1, 3).reshape(B, Sq, H * Dh) @ wo

    def _B_ref(x, k_cache, v_cache, wq, wo):
        B, Sq, D = x.shape
        H, Dh = 32, 128
        q = (lambda x, *d: x.transpose(*d))((x @ wq).reshape(B, Sq, H, Dh), 0, 2, 1, 3)
        scores = jnp.einsum("bhqd,bhkd->bhqk", q, k_cache) * (Dh ** -0.5)
        p = _softmax(scores, axis=-1)
        o = jnp.einsum("bhqk,bhkd->bhqd", p, v_cache)
        return (lambda x, *d: x.transpose(*d))(o, 0, 2, 1, 3).reshape(B, Sq, H * Dh) @ wo

    a = _A_ref(A_x, A_k_cache, A_v_cache, A_wq, A_wo)
    b = _B_ref(B_x, B_k_cache, B_v_cache, B_wq, B_wo)
    return jnp.concatenate([a, b], axis=-1)
```

```python
import functools
import jax
import jax.numpy as jnp
import jax.experimental.pallas as pl
import jax.experimental.pallas.tpu as pltpu

HC = 4

@jax.jit
def pallas_concat_heads__mha_block_cached__mha_block_cached__near_ridge_kernel(
    A_x, A_k_cache, A_v_cache, A_wq, A_wo, B_x, B_k_cache, B_v_cache, B_wq, B_wo):
    B, Sq, D = A_x.shape
    _, H, Sk, Dh = A_k_cache.shape
    M = B * Sq
    NC = H // HC
    C = HC * Dh
    scale = Dh ** -0.5
    GB = 128 // Sq
    NG = B // GB

    def kernel(ax, ak, av, awq, awo, bx, bk, bv, bwq, bwo, o_ref, q_s, o_s, acc):
        m = pl.program_id(0)
        c = pl.program_id(1)

        def compute(x_ref, k_ref, v_ref, wq_ref, wo_ref):
            q = jnp.dot(x_ref[...], wq_ref[...], preferred_element_type=jnp.float32)
            q_s[...] = q.astype(jnp.bfloat16)
            r = jax.lax.broadcasted_iota(jnp.int32, (128, 128), 0) // Sq
            cc = jax.lax.broadcasted_iota(jnp.int32, (128, 128), 1) // Sk
            mask = r == cc
            for g in range(NG):
                for h in range(HC):
                    qs = q_s[g * 128:(g + 1) * 128, h * Dh:(h + 1) * Dh]
                    ks = k_ref[g * GB:(g + 1) * GB, h].reshape(128, Dh)
                    vs = v_ref[g * GB:(g + 1) * GB, h].reshape(128, Dh)
                    s = jax.lax.dot_general(qs, ks, (((1,), (1,)), ((), ())),
                                            preferred_element_type=jnp.float32) * scale
                    s = jnp.where(mask, s, -jnp.inf)
                    mx = jnp.max(s, axis=1, keepdims=True)
                    e = jnp.exp(s - mx)
                    l = jnp.sum(e, axis=1, keepdims=True)
                    p = (e / l).astype(jnp.bfloat16)
                    o = jnp.dot(p, vs, preferred_element_type=jnp.float32)
                    o_s[g * 128:(g + 1) * 128, h * Dh:(h + 1) * Dh] = o.astype(jnp.bfloat16)
            part = jnp.dot(o_s[...], wo_ref[...], preferred_element_type=jnp.float32)

            @pl.when(c == 0)
            def _():
                acc[...] = part

            @pl.when(c > 0)
            def _():
                acc[...] += part

        @pl.when(m == 0)
        def _():
            compute(ax, ak, av, awq, awo)

        @pl.when(m == 1)
        def _():
            compute(bx, bk, bv, bwq, bwo)

        @pl.when(c == NC - 1)
        def _():
            o_ref[...] = acc[...].astype(o_ref.dtype)

    def ia(m, c):
        return jnp.where(m == 0, c, NC - 1)

    def ib(m, c):
        return jnp.where(m == 1, c, 0)

    def specs(f):
        return [
            pl.BlockSpec((M, D), lambda m, c: (0, 0)),
            pl.BlockSpec((B, HC, Sk, Dh), lambda m, c: (0, f(m, c), 0, 0)),
            pl.BlockSpec((B, HC, Sk, Dh), lambda m, c: (0, f(m, c), 0, 0)),
            pl.BlockSpec((D, C), lambda m, c: (0, f(m, c))),
            pl.BlockSpec((C, D), lambda m, c: (f(m, c), 0)),
        ]

    out = pl.pallas_call(
        kernel,
        grid=(2, NC),
        in_specs=specs(ia) + specs(ib),
        out_specs=pl.BlockSpec((M, D), lambda m, c: (0, m)),
        out_shape=jax.ShapeDtypeStruct((M, 2 * D), jnp.bfloat16),
        scratch_shapes=[
            pltpu.VMEM((M, C), jnp.bfloat16),
            pltpu.VMEM((M, C), jnp.bfloat16),
            pltpu.VMEM((M, D), jnp.float32),
        ],
        compiler_params=pltpu.CompilerParams(
            dimension_semantics=("arbitrary", "arbitrary"),
            vmem_limit_bytes=100 * 1024 * 1024,
        ),
    )(A_x.reshape(M, D), A_k_cache, A_v_cache, A_wq, A_wo,
      B_x.reshape(M, D), B_k_cache, B_v_cache, B_wq, B_wo)
    return out.reshape(B, Sq, 2 * D)
```

```python
import functools
import math
import jax
import jax.numpy as jnp
import jax.experimental.pallas as pl
import jax.experimental.pallas.tpu as pltpu

HC = 4

@jax.jit
def pallas_concat_heads__mha_block_cached__mha_block_cached__near_ridge_kernel(
    A_x, A_k_cache, A_v_cache, A_wq, A_wo, B_x, B_k_cache, B_v_cache, B_wq, B_wo):
    B, Sq, D = A_x.shape
    _, H, Sk, Dh = A_k_cache.shape
    M = B * Sq
    NC = H // HC
    T = 2 * NC
    C = HC * Dh
    cexp = (Dh ** -0.5) * math.log2(math.e)
    R = 128
    GB = R // Sq
    NG = B // GB

    def kernel(ax, ak, av, awq, awo, bx, bk, bv, bwq, bwo, out_hbm,
               x_s, wq_s, k_s, v_s, wo_s, q_s, o_s, acc, out_s,
               sem_xa, sem_xb, sem_wq, sem_k, sem_v, sem_wo, sem_out):
        t = pl.program_id(0)

        def cp_xa(g):
            return pltpu.make_async_copy(ax.at[pl.ds(g * R, R)], x_s.at[0, pl.ds(g * R, R)], sem_xa.at[g])

        def cp_xb():
            return pltpu.make_async_copy(bx, x_s.at[1], sem_xb.at[0])

        def cp_out(m, g):
            return pltpu.make_async_copy(out_s.at[m, pl.ds(g * R, R)],
                                         out_hbm.at[pl.ds(g * R, R), pl.ds(m * D, D)],
                                         sem_out.at[m * NG + g])

        def by_block(c, f):
            @pl.when(c < NC)
            def _():
                f((ak, av, awq, awo), c)

            @pl.when(c >= NC)
            def _():
                f((bk, bv, bwq, bwo), c - NC)

        def cp_wq(refs, lc, slot):
            return pltpu.make_async_copy(refs[2].at[:, pl.ds(pl.multiple_of(lc * C, C), C)], wq_s.at[slot], sem_wq.at[slot])

        def cp_k(refs, lc, slot):
            return pltpu.make_async_copy(refs[0].at[:, pl.ds(lc * HC, HC)], k_s.at[slot], sem_k.at[slot])

        def cp_v(refs, lc, slot):
            return pltpu.make_async_copy(refs[1].at[:, pl.ds(lc * HC, HC)], v_s.at[slot], sem_v.at[slot])

        def cp_wo(refs, lc, slot):
            return pltpu.make_async_copy(refs[3].at[pl.ds(pl.multiple_of(lc * C, C), C), :], wo_s.at[slot], sem_wo.at[slot])

        def start(cp, c):
            by_block(c, lambda refs, lc: cp(refs, lc, c % 2).start())

        def wait(cp, c):
            cp((ak, av, awq, awo), 0, c % 2).wait()

        def piece_q(g):
            slot = t % 2
            m = t // NC
            q = jnp.dot(x_s[m, g * R:(g + 1) * R, :], wq_s[slot], preferred_element_type=jnp.float32)
            q_s[slot, g * R:(g + 1) * R, :] = q.astype(jnp.bfloat16)

        def piece_s(g, h):
            slot = (t - 1) % 2
            qs = q_s[slot, g * R:(g + 1) * R, h * Dh:(h + 1) * Dh]
            ks = k_s[slot, g * GB:(g + 1) * GB, h].reshape(R, Dh)
            s = jax.lax.dot_general(qs, ks, (((1,), (1,)), ((), ())),
                                    preferred_element_type=jnp.float32)
            r = jax.lax.broadcasted_iota(jnp.int32, (R, R), 0) // Sq
            cc = jax.lax.broadcasted_iota(jnp.int32, (R, R), 1) // Sk
            s = jnp.where(r == cc, s, -jnp.inf)
            mx = jnp.max(s, axis=1, keepdims=True)
            e = jnp.exp2((s - mx) * cexp)
            l = jnp.sum(e, axis=1, keepdims=True)
            p = (e * pl.reciprocal(l, approx=True)).astype(jnp.bfloat16)
            return p

        def piece_pv(g, h, p):
            slot = (t - 1) % 2
            vs = v_s[slot, g * GB:(g + 1) * GB, h].reshape(R, Dh)
            o = jnp.dot(p, vs, preferred_element_type=jnp.float32)
            o_s[slot, g * R:(g + 1) * R, h * Dh:(h + 1) * Dh] = o.astype(jnp.bfloat16)

        def piece_o(g):
            slot = t % 2
            first = ((t - 2) % NC) == 0
            m = (t - 2) // NC
            rows = slice(g * R, (g + 1) * R)
            part = jnp.dot(o_s[slot, rows, :], wo_s[slot], preferred_element_type=jnp.float32)
            a = jnp.where(first, 0.0, acc[rows, :]) + part
            acc[rows, :] = a
            out_s[m, rows, :] = a.astype(out_s.dtype)

        @pl.when(t == 0)
        def _():
            cp_wq((ak, av, awq, awo), 0, 0).start()
            cp_xa(0).start()
            cp_xa(1).start()
            wait(cp_wq, 0)
            cp_xa(0).wait()
            for g in range(2, NG):
                cp_xa(g).start()
            piece_q(0)
            for g in range(1, 4):
                cp_xa(g).wait()
            cp_wq((ak, av, awq, awo), 1, 1).start()
            cp_k((ak, av, awq, awo), 0, 0).start()
            cp_v((ak, av, awq, awo), 0, 0).start()
            for g in range(1, 4):
                piece_q(g)
            for g in range(4, NG):
                cp_xa(g).wait()
            for g in range(4, NG):
                piece_q(g)

        @pl.when(t == 1)
        def _():
            wait(cp_wq, 1)
            wait(cp_k, 0)
            wait(cp_v, 0)
            cp_k((ak, av, awq, awo), 1, 1).start()
            cp_v((ak, av, awq, awo), 1, 1).start()
            cp_wq((ak, av, awq, awo), 2, 0).start()
            cp_wo((ak, av, awq, awo), 0, 0).start()
            for g in range(NG):
                ps = [piece_s(g, h) for h in range(HC)]
                piece_q(g)
                for h in range(HC):
                    piece_pv(g, h, ps[h])

        @pl.when(jnp.logical_and(t >= 2, t < T))
        def _():
            wait(cp_wq, t)
            wait(cp_k, t - 1)
            wait(cp_v, t - 1)
            wait(cp_wo, t - 2)

            @pl.when(t == NC)
            def _():
                cp_xb().wait()

            start(cp_k, t)
            start(cp_v, t)

            @pl.when(t + 1 < T)
            def _():
                start(cp_wq, t + 1)
            start(cp_wo, t - 1)

            @pl.when(t == 3)
            def _():
                cp_xb().start()
            H2 = HC // 2
            for g in range(NG):
                ps = [piece_s(g, h) for h in range(H2)]
                piece_q(g)
                for h in range(H2):
                    piece_pv(g, h, ps[h])
                ps = [piece_s(g, h) for h in range(H2, HC)]
                piece_o(g)

                @pl.when(t == NC + 1)
                def _():
                    cp_out(0, g).start()
                for h in range(H2, HC):
                    piece_pv(g, h, ps[h - H2])

        @pl.when(t == T)
        def _():
            wait(cp_k, T - 1)
            wait(cp_v, T - 1)
            wait(cp_wo, T - 2)
            cp_wo((bk, bv, bwq, bwo), NC - 1, (T - 1) % 2).start()
            for g in range(NG):
                ps = [piece_s(g, h) for h in range(HC)]
                piece_o(g)
                for h in range(HC):
                    piece_pv(g, h, ps[h])

        @pl.when(t == T + 1)
        def _():
            wait(cp_wo, T - 1)
            for g in range(NG):
                piece_o(g)
                cp_out(1, g).start()
            for m in range(2):
                for g in range(NG):
                    cp_out(m, g).wait()

    any_spec = pl.BlockSpec(memory_space=pl.ANY)
    out = pl.pallas_call(
        kernel,
        grid=(T + 2,),
        in_specs=[any_spec] * 10,
        out_specs=any_spec,
        out_shape=jax.ShapeDtypeStruct((M, 2 * D), jnp.bfloat16),
        scratch_shapes=[
            pltpu.VMEM((2, M, D), jnp.bfloat16),
            pltpu.VMEM((2, D, C), jnp.bfloat16),
            pltpu.VMEM((2, B, HC, Sk, Dh), jnp.bfloat16),
            pltpu.VMEM((2, B, HC, Sk, Dh), jnp.bfloat16),
            pltpu.VMEM((2, C, D), jnp.bfloat16),
            pltpu.VMEM((2, M, C), jnp.bfloat16),
            pltpu.VMEM((2, M, C), jnp.bfloat16),
            pltpu.VMEM((M, D), jnp.float32),
            pltpu.VMEM((2, M, D), jnp.bfloat16),
            pltpu.SemaphoreType.DMA((NG,)),
            pltpu.SemaphoreType.DMA((1,)),
            pltpu.SemaphoreType.DMA((2,)),
            pltpu.SemaphoreType.DMA((2,)),
            pltpu.SemaphoreType.DMA((2,)),
            pltpu.SemaphoreType.DMA((2,)),
            pltpu.SemaphoreType.DMA((2 * NG,)),
        ],
        compiler_params=pltpu.CompilerParams(
            dimension_semantics=("arbitrary",),
            vmem_limit_bytes=100 * 1024 * 1024,
            disable_bounds_checks=True,
        ),
    )(A_x.reshape(M, D), A_k_cache, A_v_cache, A_wq, A_wo,
      B_x.reshape(M, D), B_k_cache, B_v_cache, B_wq, B_wo)
    return out.reshape(B, Sq, 2 * D)
```

```python
import math

import jax
import jax.numpy as jnp
import jax.experimental.pallas as pl
import jax.experimental.pallas.tpu as pltpu

HC = 4
R = 128


@jax.jit
def pallas_concat_heads__mha_block_cached__mha_block_cached__near_ridge_kernel(
    A_x: jax.Array,
    A_k_cache: jax.Array,
    A_v_cache: jax.Array,
    A_wq: jax.Array,
    A_wo: jax.Array,
    B_x: jax.Array,
    B_k_cache: jax.Array,
    B_v_cache: jax.Array,
    B_wq: jax.Array,
    B_wo: jax.Array,
):
    B, Sq, D = A_x.shape
    _, H, Sk, Dh = A_k_cache.shape
    assert Sq == Sk and R % Sq == 0 and Dh == R and H % HC == 0
    M = B * Sq
    NC = H // HC
    T = 2 * NC
    C = HC * Dh
    GB = R // Sq
    NG = B // GB
    assert B % GB == 0 and NG % 2 == 0 and NG >= 4 and NC >= 4
    cexp = (Dh ** -0.5) * math.log2(math.e)

    def kernel(ax, ak, av, awq, awo, bx, bk, bv, bwq, bwo, out_hbm,
               x_s, wq_s, k_s, v_s, wo_s, q_s, o_s, acc, out_s,
               sem_xa, sem_xb, sem_wq, sem_k, sem_v, sem_wo, sem_out, sem_h):
        t = pl.program_id(0)
        a_refs = (ak, av, awq, awo)
        b_refs = (bk, bv, bwq, bwo)

        def cp_xa(g):
            return pltpu.make_async_copy(
                ax.at[pl.ds(g * R, R)], x_s.at[0, pl.ds(g * R, R)], sem_xa.at[g])

        def cp_xb():
            return pltpu.make_async_copy(bx, x_s.at[1], sem_xb.at[0])

        def cp_out(m, g):
            return pltpu.make_async_copy(
                out_s.at[m, pl.ds(g * R, R)],
                out_hbm.at[pl.ds(g * R, R), pl.ds(m * D, D)],
                sem_out.at[m * NG + g])

        def cp_wq(refs, lc, slot):
            return pltpu.make_async_copy(
                refs[2].at[:, pl.ds(pl.multiple_of(lc * C, C), C)],
                wq_s.at[slot], sem_wq.at[slot])

        def cp_k(refs, lc, slot):
            return pltpu.make_async_copy(
                refs[0].at[:, pl.ds(lc * HC, HC)], k_s.at[slot], sem_k.at[slot])

        def cp_v(refs, lc, slot):
            return pltpu.make_async_copy(
                refs[1].at[:, pl.ds(lc * HC, HC)], v_s.at[slot], sem_v.at[slot])

        def cp_wo(refs, lc, slot):
            return pltpu.make_async_copy(
                refs[3].at[pl.ds(pl.multiple_of(lc * C, C), C), :],
                wo_s.at[slot], sem_wo.at[slot])

        def cp_kv0(src_ref, dst_ref, half, j):
            hb = B // 2
            return pltpu.make_async_copy(
                src_ref.at[pl.ds(half * hb, hb), pl.ds(0, HC)],
                dst_ref.at[0, pl.ds(half * hb, hb)], sem_h.at[j])

        def start(cp, c):
            @pl.when(c < NC)
            def _():
                cp(a_refs, c, c % 2).start()

            @pl.when(c >= NC)
            def _():
                cp(b_refs, c - NC, c % 2).start()

        def wait(cp, c):
            cp(a_refs, 0, c % 2).wait()

        def piece_q(g):
            slot = t % 2
            m = t // NC
            q = jnp.dot(x_s[m, g * R:(g + 1) * R, :], wq_s[slot],
                        preferred_element_type=jnp.float32)
            q_s[slot, g * R:(g + 1) * R, :] = q.astype(jnp.bfloat16)

        def piece_s(g, h):
            slot = (t - 1) % 2
            qs = q_s[slot, g * R:(g + 1) * R, h * Dh:(h + 1) * Dh]
            ks = k_s[slot, g * GB:(g + 1) * GB, h].reshape(R, Dh)
            s = jax.lax.dot_general(qs, ks, (((1,), (1,)), ((), ())),
                                    preferred_element_type=jnp.float32)
            r = jax.lax.broadcasted_iota(jnp.int32, (R, R), 0) // Sq
            cc = jax.lax.broadcasted_iota(jnp.int32, (R, R), 1) // Sk
            s = jnp.where(r == cc, s, -jnp.inf)
            mx = jnp.max(s, axis=1, keepdims=True)
            e = jnp.exp2((s - mx) * cexp)
            l = jnp.sum(e, axis=1, keepdims=True)
            return (e * pl.reciprocal(l, approx=True)).astype(jnp.bfloat16)

        def piece_pv(g, h, p):
            slot = (t - 1) % 2
            vs = v_s[slot, g * GB:(g + 1) * GB, h].reshape(R, Dh)
            o = jnp.dot(p, vs, preferred_element_type=jnp.float32)
            o_s[slot, g * R:(g + 1) * R, h * Dh:(h + 1) * Dh] = o.astype(jnp.bfloat16)

        def piece_o(g):
            slot = t % 2
            first = ((t - 2) % NC) == 0
            m = (t - 2) // NC
            rows = slice(g * R, (g + 1) * R)
            part = jnp.dot(o_s[slot, rows, :], wo_s[slot],
                           preferred_element_type=jnp.float32)
            a = jnp.where(first, 0.0, acc[rows, :]) + part
            acc[rows, :] = a
            out_s[m, rows, :] = a.astype(out_s.dtype)

        @pl.when(t == 0)
        def _():
            cp_wq(a_refs, 0, 0).start()
            cp_xa(0).start()
            cp_xa(1).start()
            wait(cp_wq, 0)
            cp_xa(0).wait()
            for g in range(2, NG):
                cp_xa(g).start()
            piece_q(0)
            for g in range(1, NG // 2):
                cp_xa(g).wait()
            cp_wq(a_refs, 1, 1).start()
            cp_kv0(ak, k_s, 0, 0).start()
            cp_kv0(av, v_s, 0, 1).start()
            cp_kv0(ak, k_s, 1, 2).start()
            cp_kv0(av, v_s, 1, 3).start()
            for g in range(1, NG // 2):
                piece_q(g)
            for g in range(NG // 2, NG):
                cp_xa(g).wait()
            for g in range(NG // 2, NG):
                piece_q(g)

        @pl.when(t == 1)
        def _():
            wait(cp_wq, 1)
            cp_kv0(ak, k_s, 0, 0).wait()
            cp_kv0(av, v_s, 0, 1).wait()
            cp_k(a_refs, 1, 1).start()
            cp_v(a_refs, 1, 1).start()
            cp_wq(a_refs, 2, 0).start()
            cp_wo(a_refs, 0, 0).start()
            for g in range(NG):
                if g == NG // 2:
                    cp_kv0(ak, k_s, 1, 2).wait()
                    cp_kv0(av, v_s, 1, 3).wait()
                ps = [piece_s(g, h) for h in range(HC)]
                piece_q(g)
                for h in range(HC):
                    piece_pv(g, h, ps[h])

        @pl.when(jnp.logical_and(t >= 2, t < T))
        def _():
            wait(cp_wq, t)
            wait(cp_k, t - 1)
            wait(cp_v, t - 1)
            wait(cp_wo, t - 2)

            @pl.when(t == NC)
            def _():
                cp_xb().wait()

            start(cp_k, t)
            start(cp_v, t)

            @pl.when(t + 1 < T)
            def _():
                start(cp_wq, t + 1)

            start(cp_wo, t - 1)

            @pl.when(t == 3)
            def _():
                cp_xb().start()

            for g in range(NG):
                ps = [piece_s(g, h) for h in range(HC)]
                piece_q(g)
                piece_o(g)
                for h in range(HC):
                    piece_pv(g, h, ps[h])

                @pl.when(t == NC + 1)
                def _():
                    cp_out(0, g).start()

        @pl.when(t == T)
        def _():
            wait(cp_k, T - 1)
            wait(cp_v, T - 1)
            wait(cp_wo, T - 2)
            cp_wo(b_refs, NC - 1, (T - 1) % 2).start()
            for g in range(NG):
                ps = [piece_s(g, h) for h in range(HC)]
                piece_o(g)
                for h in range(HC):
                    piece_pv(g, h, ps[h])

        @pl.when(t == T + 1)
        def _():
            wait(cp_wo, T - 1)
            for g in range(NG):
                piece_o(g)
                cp_out(1, g).start()
            for m in range(2):
                for g in range(NG):
                    cp_out(m, g).wait()

    any_spec = pl.BlockSpec(memory_space=pl.ANY)
    out = pl.pallas_call(
        kernel,
        grid=(T + 2,),
        in_specs=[any_spec] * 10,
        out_specs=any_spec,
        out_shape=jax.ShapeDtypeStruct((M, 2 * D), jnp.bfloat16),
        scratch_shapes=[
            pltpu.VMEM((2, M, D), jnp.bfloat16),
            pltpu.VMEM((2, D, C), jnp.bfloat16),
            pltpu.VMEM((2, B, HC, Sk, Dh), jnp.bfloat16),
            pltpu.VMEM((2, B, HC, Sk, Dh), jnp.bfloat16),
            pltpu.VMEM((2, C, D), jnp.bfloat16),
            pltpu.VMEM((2, M, C), jnp.bfloat16),
            pltpu.VMEM((2, M, C), jnp.bfloat16),
            pltpu.VMEM((M, D), jnp.float32),
            pltpu.VMEM((2, M, D), jnp.bfloat16),
            pltpu.SemaphoreType.DMA((NG,)),
            pltpu.SemaphoreType.DMA((1,)),
            pltpu.SemaphoreType.DMA((2,)),
            pltpu.SemaphoreType.DMA((2,)),
            pltpu.SemaphoreType.DMA((2,)),
            pltpu.SemaphoreType.DMA((2,)),
            pltpu.SemaphoreType.DMA((2 * NG,)),
            pltpu.SemaphoreType.DMA((4,)),
        ],
        compiler_params=pltpu.CompilerParams(
            dimension_semantics=("arbitrary",),
            vmem_limit_bytes=100 * 1024 * 1024,
            disable_bounds_checks=True,
        ),
    )(A_x.reshape(M, D), A_k_cache, A_v_cache, A_wq, A_wo,
      B_x.reshape(M, D), B_k_cache, B_v_cache, B_wq, B_wo)
    return out.reshape(B, Sq, 2 * D)
```

```python
import math

import jax
import jax.numpy as jnp
import jax.experimental.pallas as pl
import jax.experimental.pallas.tpu as pltpu

HC = 4
R = 128


@jax.jit
def pallas_concat_heads__mha_block_cached__mha_block_cached__near_ridge_kernel(
    A_x: jax.Array,
    A_k_cache: jax.Array,
    A_v_cache: jax.Array,
    A_wq: jax.Array,
    A_wo: jax.Array,
    B_x: jax.Array,
    B_k_cache: jax.Array,
    B_v_cache: jax.Array,
    B_wq: jax.Array,
    B_wo: jax.Array,
):
    B, Sq, D = A_x.shape
    _, H, Sk, Dh = A_k_cache.shape
    assert Sq == Sk and R % Sq == 0 and Dh == R and H % HC == 0
    M = B * Sq
    NC = H // HC
    T = 2 * NC
    C = HC * Dh
    GB = R // Sq
    NG = B // GB
    assert B % GB == 0 and NG % 2 == 0 and NG >= 4 and NC >= 4
    cexp = (Dh ** -0.5) * math.log2(math.e)

    def kernel(ax, ak, av, awq, awo, bx, bk, bv, bwq, bwo, out_hbm,
               x_s, wq_s, k_s, v_s, wo_s, q_s, o_s, acc, out_s,
               sem_xa, sem_xb, sem_wq, sem_k, sem_v, sem_wo, sem_out, sem_h):
        t = pl.program_id(0)

        def par(c):
            return c % 2 if isinstance(c, int) else jax.lax.bitwise_and(c, 1)
        a_refs = (ak, av, awq, awo)
        b_refs = (bk, bv, bwq, bwo)

        def cp_xa(g):
            return pltpu.make_async_copy(
                ax.at[pl.ds(g * R, R)], x_s.at[0, pl.ds(g * R, R)], sem_xa.at[g])

        def cp_xb():
            return pltpu.make_async_copy(bx, x_s.at[1], sem_xb.at[0])

        def cp_out(m, g):
            return pltpu.make_async_copy(
                out_s.at[m, pl.ds(g * R, R)],
                out_hbm.at[pl.ds(g * R, R), pl.ds(m * D, D)],
                sem_out.at[m * NG + g])

        def cp_wq(refs, lc, slot):
            return pltpu.make_async_copy(
                refs[2].at[:, pl.ds(pl.multiple_of(lc * C, C), C)],
                wq_s.at[slot], sem_wq.at[slot])

        def cp_k(refs, lc, slot):
            return pltpu.make_async_copy(
                refs[0].at[:, pl.ds(lc * HC, HC)], k_s.at[slot], sem_k.at[slot])

        def cp_v(refs, lc, slot):
            return pltpu.make_async_copy(
                refs[1].at[:, pl.ds(lc * HC, HC)], v_s.at[slot], sem_v.at[slot])

        def cp_wo(refs, lc, slot):
            return pltpu.make_async_copy(
                refs[3].at[pl.ds(pl.multiple_of(lc * C, C), C), :],
                wo_s.at[slot], sem_wo.at[slot])

        def cp_kv0(src_ref, dst_ref, half, j):
            hb = B // 2
            return pltpu.make_async_copy(
                src_ref.at[pl.ds(half * hb, hb), pl.ds(0, HC)],
                dst_ref.at[0, pl.ds(half * hb, hb)], sem_h.at[j])

        def start(cp, c):
            @pl.when(c < NC)
            def _():
                cp(a_refs, c, par(c)).start()

            @pl.when(c >= NC)
            def _():
                cp(b_refs, c - NC, par(c)).start()

        def wait(cp, c):
            cp(a_refs, 0, par(c)).wait()

        def piece_q(g):
            slot = par(t)
            m = (t >= NC).astype(jnp.int32)
            q = jnp.dot(x_s[m, g * R:(g + 1) * R, :], wq_s[slot],
                        preferred_element_type=jnp.float32)
            q_s[slot, g * R:(g + 1) * R, :] = q.astype(jnp.bfloat16)

        def piece_s(g, h):
            slot = par(t - 1)
            qs = q_s[slot, g * R:(g + 1) * R, h * Dh:(h + 1) * Dh]
            ks = k_s[slot, g * GB:(g + 1) * GB, h].reshape(R, Dh)
            s = jax.lax.dot_general(qs, ks, (((1,), (1,)), ((), ())),
                                    preferred_element_type=jnp.float32)
            r = jax.lax.broadcasted_iota(jnp.int32, (R, R), 0) // Sq
            cc = jax.lax.broadcasted_iota(jnp.int32, (R, R), 1) // Sk
            s = jnp.where(r == cc, s, -jnp.inf)
            mx = jnp.max(s, axis=1, keepdims=True)
            e = jnp.exp2((s - mx) * cexp)
            l = jnp.sum(e, axis=1, keepdims=True)
            return (e * pl.reciprocal(l, approx=True)).astype(jnp.bfloat16)

        def piece_pv(g, h, p):
            slot = par(t - 1)
            vs = v_s[slot, g * GB:(g + 1) * GB, h].reshape(R, Dh)
            o = jnp.dot(p, vs, preferred_element_type=jnp.float32)
            o_s[slot, g * R:(g + 1) * R, h * Dh:(h + 1) * Dh] = o.astype(jnp.bfloat16)

        def piece_o(g):
            slot = par(t)
            first = jnp.logical_or(t == 2, t == NC + 2)
            m = (t >= NC + 2).astype(jnp.int32)
            rows = slice(g * R, (g + 1) * R)
            part = jnp.dot(o_s[slot, rows, :], wo_s[slot],
                           preferred_element_type=jnp.float32)
            a = jnp.where(first, 0.0, acc[rows, :]) + part
            acc[rows, :] = a
            out_s[m, rows, :] = a.astype(out_s.dtype)

        @pl.when(t == 0)
        def _():
            cp_wq(a_refs, 0, 0).start()
            cp_xa(0).start()
            cp_xa(1).start()
            wait(cp_wq, 0)
            cp_xa(0).wait()
            for g in range(2, NG):
                cp_xa(g).start()
            piece_q(0)
            for g in range(1, NG // 2):
                cp_xa(g).wait()
            cp_wq(a_refs, 1, 1).start()
            cp_kv0(ak, k_s, 0, 0).start()
            cp_kv0(av, v_s, 0, 1).start()
            cp_kv0(ak, k_s, 1, 2).start()
            cp_kv0(av, v_s, 1, 3).start()
            for g in range(1, NG // 2):
                piece_q(g)
            for g in range(NG // 2, NG):
                cp_xa(g).wait()
            for g in range(NG // 2, NG):
                piece_q(g)

        @pl.when(t == 1)
        def _():
            wait(cp_wq, 1)
            cp_kv0(ak, k_s, 0, 0).wait()
            cp_kv0(av, v_s, 0, 1).wait()
            cp_k(a_refs, 1, 1).start()
            cp_v(a_refs, 1, 1).start()
            cp_wq(a_refs, 2, 0).start()
            cp_wo(a_refs, 0, 0).start()
            for g in range(NG):
                if g == NG // 2:
                    cp_kv0(ak, k_s, 1, 2).wait()
                    cp_kv0(av, v_s, 1, 3).wait()
                ps = [piece_s(g, h) for h in range(HC)]
                piece_q(g)
                for h in range(HC):
                    piece_pv(g, h, ps[h])

        @pl.when(jnp.logical_and(t >= 2, t < T))
        def _():
            wait(cp_wq, t)
            wait(cp_k, t - 1)
            wait(cp_v, t - 1)
            wait(cp_wo, t - 2)

            @pl.when(t == NC)
            def _():
                cp_xb().wait()

            start(cp_k, t)
            start(cp_v, t)

            @pl.when(t + 1 < T)
            def _():
                start(cp_wq, t + 1)

            start(cp_wo, t - 1)

            @pl.when(t == 3)
            def _():
                cp_xb().start()

            for g in range(NG):
                ps = [piece_s(g, h) for h in range(HC)]
                piece_q(g)
                piece_o(g)
                for h in range(HC):
                    piece_pv(g, h, ps[h])

                @pl.when(t == NC + 1)
                def _():
                    cp_out(0, g).start()

        @pl.when(t == T)
        def _():
            wait(cp_k, T - 1)
            wait(cp_v, T - 1)
            wait(cp_wo, T - 2)
            cp_wo(b_refs, NC - 1, (T - 1) % 2).start()
            for g in range(NG):
                ps = [piece_s(g, h) for h in range(HC)]
                piece_o(g)
                for h in range(HC):
                    piece_pv(g, h, ps[h])

        @pl.when(t == T + 1)
        def _():
            wait(cp_wo, T - 1)
            for g in range(NG):
                piece_o(g)
                cp_out(1, g).start()
            for m in range(2):
                for g in range(NG):
                    cp_out(m, g).wait()

    any_spec = pl.BlockSpec(memory_space=pl.ANY)
    out = pl.pallas_call(
        kernel,
        grid=(T + 2,),
        in_specs=[any_spec] * 10,
        out_specs=any_spec,
        out_shape=jax.ShapeDtypeStruct((M, 2 * D), jnp.bfloat16),
        scratch_shapes=[
            pltpu.VMEM((2, M, D), jnp.bfloat16),
            pltpu.VMEM((2, D, C), jnp.bfloat16),
            pltpu.VMEM((2, B, HC, Sk, Dh), jnp.bfloat16),
            pltpu.VMEM((2, B, HC, Sk, Dh), jnp.bfloat16),
            pltpu.VMEM((2, C, D), jnp.bfloat16),
            pltpu.VMEM((2, M, C), jnp.bfloat16),
            pltpu.VMEM((2, M, C), jnp.bfloat16),
            pltpu.VMEM((M, D), jnp.float32),
            pltpu.VMEM((2, M, D), jnp.bfloat16),
            pltpu.SemaphoreType.DMA((NG,)),
            pltpu.SemaphoreType.DMA((1,)),
            pltpu.SemaphoreType.DMA((2,)),
            pltpu.SemaphoreType.DMA((2,)),
            pltpu.SemaphoreType.DMA((2,)),
            pltpu.SemaphoreType.DMA((2,)),
            pltpu.SemaphoreType.DMA((2 * NG,)),
            pltpu.SemaphoreType.DMA((4,)),
        ],
        compiler_params=pltpu.CompilerParams(
            dimension_semantics=("arbitrary",),
            vmem_limit_bytes=100 * 1024 * 1024,
            disable_bounds_checks=True,
        ),
    )(A_x.reshape(M, D), A_k_cache, A_v_cache, A_wq, A_wo,
      B_x.reshape(M, D), B_k_cache, B_v_cache, B_wq, B_wo)
    return out.reshape(B, Sq, 2 * D)
```

```python
import math

import jax
import jax.numpy as jnp
import jax.experimental.pallas as pl
import jax.experimental.pallas.tpu as pltpu

HC = 4
R = 128


@jax.jit
def pallas_concat_heads__mha_block_cached__mha_block_cached__near_ridge_kernel(
    A_x: jax.Array,
    A_k_cache: jax.Array,
    A_v_cache: jax.Array,
    A_wq: jax.Array,
    A_wo: jax.Array,
    B_x: jax.Array,
    B_k_cache: jax.Array,
    B_v_cache: jax.Array,
    B_wq: jax.Array,
    B_wo: jax.Array,
):
    B, Sq, D = A_x.shape
    _, H, Sk, Dh = A_k_cache.shape
    assert Sq == Sk and R % Sq == 0 and Dh == R and H % HC == 0
    M = B * Sq
    NC = H // HC
    T = 2 * NC
    C = HC * Dh
    GB = R // Sq
    NG = B // GB
    assert B % GB == 0 and NG % 2 == 0 and NG >= 4 and NC >= 4
    cexp = (Dh ** -0.5) * math.log2(math.e)

    def kernel(ax, ak, av, awq, awo, bx, bk, bv, bwq, bwo, out_hbm,
               x_s, wq_s, k_s, v_s, wo_s, q_s, o_s, acc, out_s,
               sem_xa, sem_xb, sem_wq, sem_k, sem_v, sem_wo, sem_out, sem_h):
        def par(c):
            return c % 2 if isinstance(c, int) else jax.lax.bitwise_and(c, 1)

        a_refs = (ak, av, awq, awo)
        b_refs = (bk, bv, bwq, bwo)

        def cp_xa(g):
            return pltpu.make_async_copy(
                ax.at[pl.ds(g * R, R)], x_s.at[0, pl.ds(g * R, R)], sem_xa.at[g])

        def cp_xb():
            return pltpu.make_async_copy(bx, x_s.at[1], sem_xb.at[0])

        def cp_out(m, g):
            return pltpu.make_async_copy(
                out_s.at[m, pl.ds(g * R, R)],
                out_hbm.at[pl.ds(g * R, R), pl.ds(m * D, D)],
                sem_out.at[m * NG + g])

        def cp_wq(refs, lc, slot):
            return pltpu.make_async_copy(
                refs[2].at[:, pl.ds(pl.multiple_of(lc * C, C), C)],
                wq_s.at[slot], sem_wq.at[slot])

        def cp_k(refs, lc, slot):
            return pltpu.make_async_copy(
                refs[0].at[:, pl.ds(lc * HC, HC)], k_s.at[slot], sem_k.at[slot])

        def cp_v(refs, lc, slot):
            return pltpu.make_async_copy(
                refs[1].at[:, pl.ds(lc * HC, HC)], v_s.at[slot], sem_v.at[slot])

        def cp_wo(refs, lc, slot):
            return pltpu.make_async_copy(
                refs[3].at[pl.ds(pl.multiple_of(lc * C, C), C), :],
                wo_s.at[slot], sem_wo.at[slot])

        def cp_kv0(src_ref, dst_ref, half, j):
            hb = B // 2
            return pltpu.make_async_copy(
                src_ref.at[pl.ds(half * hb, hb), pl.ds(0, HC)],
                dst_ref.at[0, pl.ds(half * hb, hb)], sem_h.at[j])

        def start(cp, c):
            @pl.when(c < NC)
            def _():
                cp(a_refs, c, par(c)).start()

            @pl.when(c >= NC)
            def _():
                cp(b_refs, c - NC, par(c)).start()

        def wait(cp, c):
            cp(a_refs, 0, par(c)).wait()

        def piece_q(t, g):
            slot = par(t)
            m = int(t >= NC) if isinstance(t, int) else (t >= NC).astype(jnp.int32)
            q = jnp.dot(x_s[m, g * R:(g + 1) * R, :], wq_s[slot],
                        preferred_element_type=jnp.float32)
            q_s[slot, g * R:(g + 1) * R, :] = q.astype(jnp.bfloat16)

        def piece_s(t, g, h):
            slot = par(t - 1)
            qs = q_s[slot, g * R:(g + 1) * R, h * Dh:(h + 1) * Dh]
            ks = k_s[slot, g * GB:(g + 1) * GB, h].reshape(R, Dh)
            s = jax.lax.dot_general(qs, ks, (((1,), (1,)), ((), ())),
                                    preferred_element_type=jnp.float32)
            r = jax.lax.broadcasted_iota(jnp.int32, (R, R), 0) // Sq
            cc = jax.lax.broadcasted_iota(jnp.int32, (R, R), 1) // Sk
            s = jnp.where(r == cc, s, -jnp.inf)
            mx = jnp.max(s, axis=1, keepdims=True)
            e = jnp.exp2((s - mx) * cexp)
            l = jnp.sum(e, axis=1, keepdims=True)
            return (e * pl.reciprocal(l, approx=True)).astype(jnp.bfloat16)

        def piece_pv(t, g, h, p):
            slot = par(t - 1)
            vs = v_s[slot, g * GB:(g + 1) * GB, h].reshape(R, Dh)
            o = jnp.dot(p, vs, preferred_element_type=jnp.float32)
            o_s[slot, g * R:(g + 1) * R, h * Dh:(h + 1) * Dh] = o.astype(jnp.bfloat16)

        def piece_o(t, g):
            slot = par(t)
            first = (t == 2 or t == NC + 2) if isinstance(t, int) else jnp.logical_or(t == 2, t == NC + 2)
            m = int(t >= NC + 2) if isinstance(t, int) else (t >= NC + 2).astype(jnp.int32)
            rows = slice(g * R, (g + 1) * R)
            part = jnp.dot(o_s[slot, rows, :], wo_s[slot],
                           preferred_element_type=jnp.float32)
            a = jnp.where(first, 0.0, acc[rows, :]) + part
            acc[rows, :] = a
            out_s[m, rows, :] = a.astype(out_s.dtype)

        def step_first(t=0):
            cp_wq(a_refs, 0, 0).start()
            cp_xa(0).start()
            cp_xa(1).start()
            wait(cp_wq, 0)
            cp_xa(0).wait()
            for g in range(2, NG):
                cp_xa(g).start()
            piece_q(t, 0)
            for g in range(1, NG // 2):
                cp_xa(g).wait()
            cp_wq(a_refs, 1, 1).start()
            cp_kv0(ak, k_s, 0, 0).start()
            cp_kv0(av, v_s, 0, 1).start()
            cp_kv0(ak, k_s, 1, 2).start()
            cp_kv0(av, v_s, 1, 3).start()
            for g in range(1, NG // 2):
                piece_q(t, g)
            for g in range(NG // 2, NG):
                cp_xa(g).wait()
            for g in range(NG // 2, NG):
                piece_q(t, g)

        def step_second(t=1):
            wait(cp_wq, 1)
            cp_kv0(ak, k_s, 0, 0).wait()
            cp_kv0(av, v_s, 0, 1).wait()
            cp_k(a_refs, 1, 1).start()
            cp_v(a_refs, 1, 1).start()
            cp_wq(a_refs, 2, 0).start()
            cp_wo(a_refs, 0, 0).start()
            for g in range(NG):
                if g == NG // 2:
                    cp_kv0(ak, k_s, 1, 2).wait()
                    cp_kv0(av, v_s, 1, 3).wait()
                ps = [piece_s(t, g, h) for h in range(HC)]
                piece_q(t, g)
                for h in range(HC):
                    piece_pv(t, g, h, ps[h])

        def step_steady(t, carry):
            wait(cp_wq, t)
            wait(cp_k, t - 1)
            wait(cp_v, t - 1)
            wait(cp_wo, t - 2)

            @pl.when(t == NC)
            def _():
                cp_xb().wait()

            start(cp_k, t)
            start(cp_v, t)

            @pl.when(t + 1 < T)
            def _():
                start(cp_wq, t + 1)

            start(cp_wo, t - 1)

            @pl.when(t == 3)
            def _():
                cp_xb().start()

            for g in range(NG):
                ps = [piece_s(t, g, h) for h in range(HC)]
                piece_q(t, g)
                piece_o(t, g)
                for h in range(HC):
                    piece_pv(t, g, h, ps[h])

                @pl.when(t == NC + 1)
                def _():
                    cp_out(0, g).start()
            return carry

        def step_penult(t=T):
            wait(cp_k, T - 1)
            wait(cp_v, T - 1)
            wait(cp_wo, T - 2)
            cp_wo(b_refs, NC - 1, (T - 1) % 2).start()
            for g in range(NG):
                ps = [piece_s(t, g, h) for h in range(HC)]
                piece_o(t, g)
                for h in range(HC):
                    piece_pv(t, g, h, ps[h])

        def step_last(t=T + 1):
            wait(cp_wo, T - 1)
            for g in range(NG):
                piece_o(t, g)
                cp_out(1, g).start()
            for m in range(2):
                for g in range(NG):
                    cp_out(m, g).wait()

        step_first()
        step_second()
        jax.lax.fori_loop(2, T, step_steady, 0)
        step_penult()
        step_last()

    any_spec = pl.BlockSpec(memory_space=pl.ANY)
    out = pl.pallas_call(
        kernel,
        in_specs=[any_spec] * 10,
        out_specs=any_spec,
        out_shape=jax.ShapeDtypeStruct((M, 2 * D), jnp.bfloat16),
        scratch_shapes=[
            pltpu.VMEM((2, M, D), jnp.bfloat16),
            pltpu.VMEM((2, D, C), jnp.bfloat16),
            pltpu.VMEM((2, B, HC, Sk, Dh), jnp.bfloat16),
            pltpu.VMEM((2, B, HC, Sk, Dh), jnp.bfloat16),
            pltpu.VMEM((2, C, D), jnp.bfloat16),
            pltpu.VMEM((2, M, C), jnp.bfloat16),
            pltpu.VMEM((2, M, C), jnp.bfloat16),
            pltpu.VMEM((M, D), jnp.float32),
            pltpu.VMEM((2, M, D), jnp.bfloat16),
            pltpu.SemaphoreType.DMA((NG,)),
            pltpu.SemaphoreType.DMA((1,)),
            pltpu.SemaphoreType.DMA((2,)),
            pltpu.SemaphoreType.DMA((2,)),
            pltpu.SemaphoreType.DMA((2,)),
            pltpu.SemaphoreType.DMA((2,)),
            pltpu.SemaphoreType.DMA((2 * NG,)),
            pltpu.SemaphoreType.DMA((4,)),
        ],
        compiler_params=pltpu.CompilerParams(
            vmem_limit_bytes=100 * 1024 * 1024,
            disable_bounds_checks=True,
        ),
    )(A_x.reshape(M, D), A_k_cache, A_v_cache, A_wq, A_wo,
      B_x.reshape(M, D), B_k_cache, B_v_cache, B_wq, B_wo)
    return out.reshape(B, Sq, 2 * D)
```
